```python
import os as _os
_os.environ.setdefault("JAX_PLATFORMS", "cpu")
import jax
import jax.numpy as jnp

def _softmax(x, axis=-1):
    return jax.nn.softmax(x, axis=axis)
def _gelu(x):
    return jax.nn.gelu(x, approximate=True)
def _silu(x):
    return jax.nn.silu(x)
def _sigmoid(x):
    return jax.nn.sigmoid(x)
def _layernorm(x, axis=-1, eps=1e-5):
    m = jnp.mean(x, axis=axis, keepdims=True)
    v = jnp.var(x, axis=axis, keepdims=True)
    return (x - m) / jnp.sqrt(v + eps)
def _scatter_add(tgt, idx, src, axis=0):
    return tgt.at[idx].add(src)
def _segment_sum(src, seg, n):
    return jax.ops.segment_sum(src, seg, n)
class _Rng:
    def __init__(self, key):
        self._k = key
    def _next(self):
        self._k, sub = jax.random.split(self._k)
        return sub
    def normal(self, shape):
        return jax.random.normal(self._next(), shape, dtype=jnp.bfloat16)
    def randint(self, lo, hi, shape):
        return jax.random.randint(self._next(), shape, lo, hi, dtype=jnp.int32)
    def uniform(self, shape, lo=0.0, hi=1.0):
        return jax.random.uniform(self._next(), shape, jnp.bfloat16, lo, hi)
    def permutation(self, n):
        return jax.random.permutation(self._next(), n)


kernel_name = 'interleave_layers__sliding_local_dilated__sliding_local_dilated__prompt'

def setup_inputs():
    _rng = _Rng(jax.random.key(int.from_bytes(__import__("os").urandom(4), "little")))
    _w = (lambda a: (lambda t: t.astype(jnp.bfloat16) if jnp.issubdtype(t.dtype, jnp.floating) else t)(jnp.asarray(a)))
    def _A_setup():
        B, S, D = 1, 2048, 1024
        return {
            "x": _w((lambda *s: _rng.normal(s) * 0.05)(B, S, D)),
            "wqkv": _w((lambda *s: _rng.normal(s) * 0.05)(D, 3 * D)),
            "wo": _w((lambda *s: _rng.normal(s) * 0.05)(D, D)),
        }
    _A_in = _A_setup()

    def _B_setup():
        B, S, D = 1, 2048, 1024
        return {
            "x": _w((lambda *s: _rng.normal(s) * 0.05)(B, S, D)),
            "wqkv": _w((lambda *s: _rng.normal(s) * 0.05)(D, 3 * D)),
            "wo": _w((lambda *s: _rng.normal(s) * 0.05)(D, D)),
        }
    _B_in = _B_setup()

    return {
        "A_x": _A_in["x"],
        "A_wqkv": _A_in["wqkv"],
        "A_wo": _A_in["wo"],
        "B_x": _B_in["x"],
        "B_wqkv": _B_in["wqkv"],
        "B_wo": _B_in["wo"],
    }

def reference(A_x, A_wqkv, A_wo, B_x, B_wqkv, B_wo):
    def _A_ref(x, wqkv, wo):
        B, S, D = x.shape
        H = 32; Dh = D // H
        W, dil = 8, 2
        qkv = (lambda x, *d: x.transpose(*d))((x @ wqkv).reshape(B, S, 3, H, Dh), 2, 0, 3, 1, 4)
        q, k, v = qkv[0], qkv[1], qkv[2]
        scale = Dh ** -0.5
        pos = jnp.arange(S)
        off = jnp.arange(W) * dil
        idx = pos[:, None] - off[None, :]
        mask = idx >= 0
        idx_c = jnp.where(mask, idx, 0).reshape(-1)
        kg = k[:, :, idx_c, :].reshape(B, H, S, W, Dh)
        vg = v[:, :, idx_c, :].reshape(B, H, S, W, Dh)
        logits = jnp.einsum("bhsd,bhswd->bhsw", q, kg) * scale
        logits = jnp.where(mask[None, None, :, :], logits, -1e9)
        attn = _softmax(logits, axis=-1)
        o = jnp.einsum("bhsw,bhswd->bhsd", attn, vg)
        return (lambda x, *d: x.transpose(*d))(o, 0, 2, 1, 3).reshape(B, S, D) @ wo

    def _B_ref(x, wqkv, wo):
        B, S, D = x.shape
        H = 32; Dh = D // H
        W, dil = 8, 2
        qkv = (lambda x, *d: x.transpose(*d))((x @ wqkv).reshape(B, S, 3, H, Dh), 2, 0, 3, 1, 4)
        q, k, v = qkv[0], qkv[1], qkv[2]
        scale = Dh ** -0.5
        pos = jnp.arange(S)
        off = jnp.arange(W) * dil
        idx = pos[:, None] - off[None, :]
        mask = idx >= 0
        idx_c = jnp.where(mask, idx, 0).reshape(-1)
        kg = k[:, :, idx_c, :].reshape(B, H, S, W, Dh)
        vg = v[:, :, idx_c, :].reshape(B, H, S, W, Dh)
        logits = jnp.einsum("bhsd,bhswd->bhsw", q, kg) * scale
        logits = jnp.where(mask[None, None, :, :], logits, -1e9)
        attn = _softmax(logits, axis=-1)
        o = jnp.einsum("bhsw,bhswd->bhsd", attn, vg)
        return (lambda x, *d: x.transpose(*d))(o, 0, 2, 1, 3).reshape(B, S, D) @ wo

    x = A_x
    x = x + _A_ref(_layernorm(x, axis=-1), A_wqkv, A_wo)
    x = x + _B_ref(_layernorm(x, axis=-1), B_wqkv, B_wo)
    x = x + _A_ref(_layernorm(x, axis=-1), A_wqkv, A_wo)
    x = x + _B_ref(_layernorm(x, axis=-1), B_wqkv, B_wo)
    return x
```

```python
import functools
import contextlib
import jax
import jax.numpy as jnp
from jax.experimental import pallas as pl
from jax.experimental.pallas import tpu as pltpu

S, D, H, DH, W = 2048, 1024, 32, 32, 8
T = S // 2
NB = T // 128
NP = NB // 2
NC = D // 128
G = 4
GR = D // G
HG = GR // DH
NE = NB + W - 1
KH = D // 2
HM = 3 * GR // 2
F32, BF16, U32 = jnp.float32, jnp.bfloat16, jnp.uint32
EPS = 1e-5
SCALE = DH ** -0.5
PITCH = DH + 1
QKV = (0, NB + 2 * NE)
TMP = 2 * (NB + 2 * NE)
PB = TMP + 10
OB = PB + 2
NT = OB + 7 * NP
WO0 = G * 7 * HM // 2


def lhs_operands(a11, a12, a21, a22):
    return (a11 + a22, a21 + a22, a11, a22, a11 + a12, a21 - a11, a12 - a22)


def rhs_operands(b11, b12, b21, b22):
    return (b11 + b22, b11, b12 - b22, b21 - b11, b22, b11 + b12, b21 + b22)


def make_kernel(SC=False, WQ=2, SR=64, SW=64, LNC=4, CODE=0):
    scope = jax.named_scope if SC else (lambda n: contextlib.nullcontext())

    def kernel(x_hbm, aqkv_hbm, awo_hbm, bqkv_hbm, bwo_hbm, out_hbm,
               x_raw, raw_qkv, raw_wo, wt, tmp, xs, xn, fb, vfirst, out_st, sems):
        def cols(i, n):
            return pl.ds(pl.multiple_of(i * n, n), n)

        def cp_x(c):
            return pltpu.make_async_copy(x_hbm.at[:, cols(c, 128)], x_raw.at[c], sems.at[c])

        def cp_a(g, part):
            cs = cols(part * G + g, GR)
            return pltpu.make_async_copy(aqkv_hbm.at[:, cs], raw_qkv.at[0, :, cs],
                                         sems.at[NC + 3 * g + part])

        cp_rest = [pltpu.make_async_copy(awo_hbm, raw_wo.at[0], sems.at[NC + 12]),
                   pltpu.make_async_copy(bqkv_hbm, raw_qkv.at[1], sems.at[NC + 13]),
                   pltpu.make_async_copy(bwo_hbm, raw_wo.at[1], sems.at[NC + 14])]
        for part in range(3):
            cp_a(0, part).start()
        for c in range(NC):
            cp_x(c).start()
        for g in range(1, G):
            for part in range(3):
                cp_a(g, part).start()
        for c in cp_rest:
            c.start()

        def prep_x(c, carry):
            xu = x_raw.bitcast(U32)
            cp_x(c).wait()
            for r in range(NB):
                wd = xu[c, pl.ds(r, 128, stride=NB), :]
                wd = pltpu.bitcast(pltpu.bitcast(wd, F32).T, U32)
                xs[0, r, cols(c, 128), :] = pltpu.bitcast(wd << 16, F32)
                xs[1, r, cols(c, 128), :] = pltpu.bitcast(wd & jnp.uint32(0xFFFF0000), F32)
            return carry

        def words(val):
            return pltpu.bitcast(val.astype(BF16), F32)

        def scatter_heads(t, val):
            for h in range(HG):
                tmp[t, h * PITCH:h * PITCH + DH, :] = val[h * DH:(h + 1) * DH]

        def gather_dims(t, d0, nd):
            return jnp.concatenate(
                [tmp[t, pl.ds(d, HG, stride=PITCH), :] for d in range(d0, d0 + nd)], axis=0)

        def prep_qkv(i, carry):
            l, g, c = i // (4 * G), (i // 4) % G, i % 4
            for half in range(2):
                for part in range(3):
                    scatter_heads(3 * half + part, raw_qkv[
                        l, cols(c + 4 * half, 128), cols(part * G + g, GR)].astype(F32).T)
            for s in range(3):
                quad = [gather_dims(3 * half + (s + 3 * mh) // 2, 16 * ((s + 3 * mh) % 2), 16)
                        for mh in range(2) for half in range(2)]
                for m, val in enumerate(lhs_operands(*quad)):
                    wt[l, c, cols((g * 7 + m) * 3 + s, 64), :] = words(val)
            return carry

        def prep_wo(i, carry):
            l, g = i // G, i % G
            for c in range(4):
                for mh in range(2):
                    scatter_heads(2 * c + mh, raw_wo[
                        l, cols(g, GR), (c + 4 * mh) * 128:(c + 4 * mh + 1) * 128].astype(F32))
                quad = [gather_dims(2 * c + mh, 16 * half, 16).T
                        for mh in range(2) for half in range(2)]
                for m, val in enumerate(lhs_operands(*quad)):
                    w0 = WO0 + m * (KH // 2) + c * 64
                    wt[l, g, w0:w0 + 64, :] = words(val)
            return carry

        def ln_pieces(p, z, j0, nj):
            zr = pl.multiple_of(z * 16, 16)
            st0 = 7 * KH

            def block(j, a):
                return xs[p, 2 * j + a].reshape(D // 8, 8, 128)

            def stat(j, i):
                return pltpu.bitcast(xn[p, j, st0 + 16 * i:st0 + 16 * (i + 1), :], F32)

            def put_stat(j, i, val):
                xn[p, j, pl.ds(zr + st0 + 16 * i, 16), :] = pltpu.bitcast(
                    jnp.broadcast_to(val, (8, 128)), BF16)

            def mean(j, a):
                m = jnp.sum(block(j, a), axis=0)
                put_stat(j, a, jnp.sum(m, axis=0, keepdims=True) * (1.0 / D))

            def var(j, a):
                c = block(j, a) - stat(j, a)[None]
                v = jnp.sum(jnp.sum(c * c, axis=0), axis=0, keepdims=True) * (1.0 / D)
                put_stat(j, 2 + a, jax.lax.rsqrt(v + EPS))

            def norm(j, i):
                n = KH // LNC
                quad = []
                for kh in range(2):
                    for a in range(2):
                        x = xs[p, 2 * j + a, kh * KH + i * n:kh * KH + (i + 1) * n, :]
                        x = (x.reshape(n // 8, 8, 128) - stat(j, a)[None]) * stat(j, 2 + a)[None]
                        quad.append(x.reshape(n, 128))
                for m, val in enumerate(rhs_operands(*quad)):
                    xn[p, j, pl.ds(zr + m * KH + i * n, n), :] = val.astype(BF16)

            pieces = []
            for j in [j0 + i for i in range(nj)]:
                pieces += [functools.partial(f, j, a) for f in (mean, var) for a in range(2)]
                pieces += [functools.partial(norm, j, i) for i in range(LNC)]
            return pieces

        def att_pieces(g, z, par):
            q0 = QKV[par]
            k0, v0 = q0 + NB, q0 + NB + NE
            lane0 = jax.lax.broadcasted_iota(jnp.int32, (8, 128), 1) == 0

            def qk(r, w0):
                acc = {}
                for d in range(DH):
                    rs = slice(8 * d, 8 * d + 8)
                    q = fb[q0 + r, rs, :]
                    for w in range(w0, w0 + WQ):
                        t = q * fb[k0 + r - w + W - 1, rs, :]
                        acc[w] = t if d == 0 else acc[w] + t
                lg = [jnp.where(lane0, -1e9, acc[w] * SCALE) if w > r else acc[w] * SCALE
                      for w in range(w0, w0 + WQ)]
                fb[z + PB + r % 2, w0 * 8:(w0 + WQ) * 8, :] = jnp.concatenate(lg, axis=0)

            def softmax(r):
                lg = [fb[PB + r % 2, w * 8:w * 8 + 8, :] for w in range(W)]
                m = functools.reduce(jnp.maximum, lg)
                e = [jnp.exp(t - m) for t in lg]
                inv = 1.0 / functools.reduce(jnp.add, e)
                fb[z + PB + r % 2, 64:128, :] = jnp.concatenate([t * inv for t in e], axis=0)

            def pv(j, c):
                quad = []
                for kh in range(2):
                    rs = slice(kh * 128 + 16 * c, kh * 128 + 16 * c + 16)
                    v = [fb[v0 + 2 * j + e, rs, :].reshape(2, 8, 128) for e in range(W + 1)]
                    for a in range(2):
                        o = None
                        for w in range(W):
                            t = v[a - w + W - 1] * fb[PB + a, 64 + w * 8:72 + w * 8, :][None]
                            o = t if o is None else o + t
                        quad.append(o.reshape(16, 128))
                for m, val in enumerate(rhs_operands(*quad)):
                    fb[z + OB + 7 * j + m, cols(8 * g + c, 8), :] = words(val)

            pieces = []
            for j in range(NP):
                for r in (2 * j, 2 * j + 1):
                    pieces += [functools.partial(qk, r, w0) for w0 in range(0, W, WQ)]
                    pieces.append(functools.partial(softmax, r))
                pieces += [functools.partial(pv, j, c) for c in range(8)]
            return pieces

        def spread(pieces, slots):
            state = [0, 0]

            def fill():
                state[0] += 1
                while state[1] < min(len(pieces), int(state[0] * len(pieces) / slots + 0.5)):
                    pieces[state[1]]()
                    state[1] += 1
            return fill

        def run(pieces):
            for f in pieces:
                f()

        def lhs(l, rows):
            return jnp.concatenate(
                [pltpu.bitcast(wt[l, c, rows, :], BF16) for c in range(4)], axis=1)

        def qkv_step(l, p, g, par, att, ln):
            q0 = QKV[par]
            k0, v0 = q0 + NB, q0 + NB + NE
            fill_att = spread(att, NP * 7 * (HM // SR))
            fill_ln = spread(ln, NP * 7)
            lane0 = jax.lax.broadcasted_iota(jnp.int32, (SR, 128), 1) == 0

            def final(row, r, val):
                part, rr = row // GR, slice(row % GR, row % GR + SR)
                if part == 0:
                    fb[q0 + r, rr, :] = val
                elif part == 1:
                    fb[k0 + W - 1 + r, rr, :] = val
                    if r > 0:
                        fb[k0 + r - 1, rr, :] = pltpu.roll(val, 1, 1)
                else:
                    fb[v0 + W - 1 + r, rr, :] = val
                    if r == 0:
                        vfirst[g, rr, :] = jnp.where(p == 0, val, vfirst[g, rr, :])
                    else:
                        fb[v0 + r - 1, rr, :] = jnp.where(
                            lane0, vfirst[g, rr, :], pltpu.roll(val, 1, 1))

            for j in range(NP):
                for m in (0, 1, 2, 5, 3, 4, 6):
                    res = jnp.dot(lhs(l, cols(g * 7 + m, HM // 2)),
                                  xn[p, j, m * KH:(m + 1) * KH, :], preferred_element_type=F32)
                    for s0 in range(0, HM, SR):
                        val = res[s0:s0 + SR]
                        t1, t2, t3, tx, ty = [
                            (TMP + 2 * t + s0 // GR, slice(s0 % GR, s0 % GR + SR), slice(None))
                            for t in range(5)]
                        if m == 0:
                            fb[t1] = val
                        elif m == 1:
                            fb[t2] = val
                        elif m == 2:
                            fb[tx] = fb[t1] - fb[t2] + val
                            fb[t3] = val
                        elif m == 5:
                            final(HM + s0, 2 * j + 1, fb[tx] + val)
                        elif m == 3:
                            final(HM + s0, 2 * j, fb[t2] + val)
                            fb[ty] = fb[t1] + val
                        elif m == 4:
                            final(s0, 2 * j + 1, fb[t3] + val)
                            fb[ty] = fb[ty] - val
                        else:
                            final(s0, 2 * j, fb[ty] + val)
                        fill_att()
                    fill_ln()

        feeds = (((0, 0, 1), (1, 1, 1)), ((1, 0, 1), (1, 1, -1)), ((0, 1, 1), (1, 1, 1)),
                 ((0, 0, 1), (1, 0, 1)), ((0, 0, -1), (0, 1, 1)), ((1, 1, 1),), ((0, 0, 1),))

        def wo_step(l, p):
            for j in range(NP):
                for m in range(7):
                    w0 = WO0 + m * (KH // 2)
                    res = jnp.dot(lhs(l, slice(w0, w0 + KH // 2)),
                                  pltpu.bitcast(fb[OB + 7 * j + m], BF16),
                                  preferred_element_type=F32)
                    for s0 in range(0, KH, SW):
                        for mh, a, sign in feeds[m]:
                            ix = (p, 2 * j + a, slice(mh * KH + s0, mh * KH + s0 + SW), slice(None))
                            xs[ix] = xs[ix] + res[s0:s0 + SW] if sign > 0 else xs[ix] - res[s0:s0 + SW]

        def prep_a_group(g):
            for part in range(3):
                cp_a(g, part).wait()
            jax.lax.fori_loop(4 * g, 4 * g + 4, prep_qkv, 0)

        vfirst[...] = jnp.zeros_like(vfirst)
        fb[QKV[1]:TMP] = jnp.zeros((TMP - QKV[1], GR, 128), F32)
        with scope("pq0"):
            prep_a_group(0)
        with scope("prep_x"):
            jax.lax.fori_loop(0, NC, prep_x, 0)
        with scope("ln0"):
            def ln0(j, carry):
                run(ln_pieces(0, 0, j, 1))
                return carry
            jax.lax.fori_loop(0, NP, ln0, 0)

        def body(i, carry):
            u, h = i // 2, i % 2
            p = u % 2
            l = (u // 2) % 2
            z = (i * i) // 512

            @pl.when(i == 1)
            def _():
                with scope("pq1"):
                    for g in (2, 3):
                        for part in range(3):
                            cp_a(g, part).wait()

            @pl.when(i == 2)
            def _():
                with scope("po"):
                    for c in cp_rest:
                        c.wait()
                    jax.lax.fori_loop(0, 2 * G, prep_wo, 0)

            @pl.when(jnp.logical_or(i == 1, i == 2))
            def _():
                with scope("pq"):
                    jax.lax.fori_loop(8 * i, 16 * i, prep_qkv, 0)

            @pl.when(i < 16)
            def _():
                with scope("sE"):
                    qkv_step(l, p, 2 * h, 0, att_pieces(3 - 2 * h, z, 1), [])

            @pl.when(i == 16)
            def _():
                with scope("tail_att"):
                    run(att_pieces(G - 1, 0, 1))

            @pl.when(jnp.logical_and(h == 0, i > 0))
            def _():
                with scope("sW"):
                    wo_step(((u - 1) // 2) % 2, 1 - p)

            @pl.when(i == 0)
            def _():
                with scope("pq0"):
                    prep_a_group(1)

            @pl.when(i < 16)
            def _():
                with scope("sO"):
                    qkv_step(l, p, 2 * h + 1, 1, att_pieces(2 * h, z, 0),
                             ln_pieces(1 - p, z, h * (NP // 2), NP // 2))
            return carry
        jax.lax.fori_loop(0, 17, body, 0)

        def cp_o(c):
            return pltpu.make_async_copy(out_st.at[c], out_hbm.at[:, cols(c, 128)], sems.at[c])

        def emit(c, carry):
            ou = out_st.bitcast(U32)
            for r in range(NB):
                ev = xs[0, r, cols(c, 128), :].astype(BF16).astype(F32)
                od = xs[1, r, cols(c, 128), :].astype(BF16).astype(F32)
                wd = (pltpu.bitcast(ev, U32) >> 16) | pltpu.bitcast(od, U32)
                ou[c, pl.ds(r, 128, stride=NB), :] = pltpu.bitcast(pltpu.bitcast(wd, F32).T, U32)
            cp_o(c).start()
            return carry
        with scope("emit"):
            jax.lax.fori_loop(0, NC, emit, 0)
        for c in range(NC):
            cp_o(c).wait()

    scratch = [
        pltpu.VMEM((NC, S, 128), BF16),
        pltpu.VMEM((2, D, 3 * D), BF16),
        pltpu.VMEM((2, D, D), BF16),
        pltpu.VMEM((2, 4, WO0 + 7 * KH // 2, 128), F32),
        pltpu.VMEM((8, HG * PITCH, 128), F32),
        pltpu.VMEM((2, NB, D, 128), F32),
        pltpu.VMEM((2, NP, 7 * KH + 64, 128), BF16),
        pltpu.VMEM((NT, GR, 128), F32),
        pltpu.VMEM((G, GR, 128), F32),
        pltpu.VMEM((NC, S, 128), BF16),
        pltpu.SemaphoreType.DMA((24,)),
    ]

    @jax.jit
    def run_kernel(A_x, A_wqkv, A_wo, B_x, B_wqkv, B_wo):
        any_spec = pl.BlockSpec(memory_space=pl.ANY)
        out = pl.pallas_call(
            kernel,
            out_shape=jax.ShapeDtypeStruct((S, D), BF16),
            in_specs=[any_spec] * 5,
            out_specs=any_spec,
            scratch_shapes=scratch,
            compiler_params=pltpu.CompilerParams(vmem_limit_bytes=112 * 1024 * 1024),
        )(A_x.reshape(S, D), A_wqkv, A_wo, B_wqkv, B_wo)
        return out.reshape(1, S, D)
    return run_kernel


_run = make_kernel()


@jax.jit
def pallas_interleave_layers__sliding_local_dilated__sliding_local_dilated__prompt_kernel(
    A_x: jax.Array,
    A_wqkv: jax.Array,
    A_wo: jax.Array,
    B_x: jax.Array,
    B_wqkv: jax.Array,
    B_wo: jax.Array,
):
    return _run(A_x, A_wqkv, A_wo, B_x, B_wqkv, B_wo)
```

```python
import functools

import jax
import jax.numpy as jnp
from jax.experimental import pallas as pl
from jax.experimental.pallas import tpu as pltpu

S, D, H, DH, W = 2048, 1024, 32, 32, 8
T = S // 2
NB = T // 128
NP = NB // 2
NC = D // 128
G = 4
GR = D // G
HG = GR // DH
NE = NB + W - 1
KH = D // 2
HM = 3 * GR // 2
F32, BF16, U32 = jnp.float32, jnp.bfloat16, jnp.uint32
EPS = 1e-5
SCALE = DH ** -0.5
ROWS = ((1, 0), (0, 0), (0, 1), (1, 1), (2, 0), (2, 1))
PITCH = DH + 1
Q0, K0, V0 = 0, NB, NB + NE
TMP = NB + 2 * NE
PB = TMP + 10
OB = PB + 2
NT = OB + 7 * NP // 2
XN0 = 2 * D
ST0 = XN0 + 7 * KH // 2
WO0 = G * 7 * HM // 2


def lhs_operands(a11, a12, a21, a22):
    return (a11 + a22, a21 + a22, a11, a22, a11 + a12, a21 - a11, a12 - a22)


def rhs_operands(b11, b12, b21, b22):
    return (b11 + b22, b11, b12 - b22, b21 - b11, b22, b11 + b12, b21 + b22)


WQ = 4
SR, SW = 32, 32
LNS, LNC = 4, 32
RS, RC = 4, 16
PU = 4


def kernel(x_hbm, aqkv_hbm, awo_hbm, bqkv_hbm, bwo_hbm, out_hbm,
           x_raw, raw_qkv, raw_wo, wt, tmp, xs, fb0, fb1, prob, moments, vfirst, out_st, sems):
    def cols(i, n):
        return pl.ds(i * n if isinstance(i, int) else pl.multiple_of(i * n, n), n)

    def cp_x(c):
        return pltpu.make_async_copy(x_hbm.at[:, cols(c, 128)], x_raw.at[c], sems.at[c])

    def cp_a(g, part):
        cs = cols(part * G + g, GR)
        return pltpu.make_async_copy(aqkv_hbm.at[:, cs], raw_qkv.at[0, :, cs],
                                     sems.at[NC + 3 * g + part])

    cp_rest = [pltpu.make_async_copy(awo_hbm, raw_wo.at[0], sems.at[NC + 12]),
               pltpu.make_async_copy(bqkv_hbm, raw_qkv.at[1], sems.at[NC + 13]),
               pltpu.make_async_copy(bwo_hbm, raw_wo.at[1], sems.at[NC + 14])]
    for c in range(NC):
        cp_x(c).start()
    for g in range(G):
        for part in range(3):
            cp_a(g, part).start()
    for c in cp_rest:
        c.start()

    def x_rows(r0, n):
        return pl.ds(r0 if isinstance(r0, int) else pl.multiple_of(r0, 8), n)

    def x_get(p, j, r0, n):
        return xs[p, j, x_rows(r0, n), :]

    def x_put(p, j, r0, val):
        xs[p, j, x_rows(r0, val.shape[0]), :] = val

    def lane_mean(v, n):
        return jnp.broadcast_to(jnp.sum(v, axis=0, keepdims=True) * (1.0 / n), (8, 128))

    def prep_x(c, carry, first=False):
        xu = x_raw.bitcast(U32)
        cp_x(c).wait()
        for r in range(NB):
            j, a = r // 2, r % 2
            wd = xu[c, pl.ds(r, 128, stride=NB), :]
            for p, val in enumerate(halves(pltpu.bitcast(wd, F32).T)):
                x_put(p, j, a * D + c * 128, val)
                val = val.reshape(16, 8, 128)
                if first:
                    shift = lane_mean(jnp.sum(val, axis=0), 128)
                    moments[p, r, 2] = shift
                else:
                    shift = moments[p, r, 2]
                dv = val - shift[None]
                for i, t in enumerate((jnp.sum(dv, axis=0), jnp.sum(dv * dv, axis=0))):
                    moments[p, r, i] = t if first else moments[p, r, i] + t
        return carry

    def first_norm(i, carry):
        p, j = i // NP, i % NP
        for a in range(2):
            m = lane_mean(moments[p, 2 * j + a, 0], D)
            v = jnp.maximum(lane_mean(moments[p, 2 * j + a, 1], D) - m * m, 0.0)
            x_put(p, j, ST0 + 8 * a, moments[p, 2 * j + a, 2] + m)
            x_put(p, j, ST0 + 8 * (2 + a), jax.lax.rsqrt(v + EPS))
        run(ln_pieces(p, 0, j, 1, RC)[1][-RC:])
        return carry

    def words(val):
        return pltpu.bitcast(val.astype(BF16), F32)

    def halves(wd):
        wd = pltpu.bitcast(wd, U32)
        return (pltpu.bitcast(wd << 16, F32),
                pltpu.bitcast(wd & jnp.uint32(0xFFFF0000), F32))

    def pack(lo, hi):
        lo, hi = (pltpu.bitcast(t.astype(BF16).astype(F32), U32) for t in (lo, hi))
        return pltpu.bitcast((lo >> 16) | hi, F32)

    def scatter_heads(t, val):
        for h in range(HG):
            tmp[t, h * PITCH:h * PITCH + DH, :] = val[h * DH:(h + 1) * DH]

    def gather_dims(t, half):
        return jnp.concatenate([tmp[t, pl.ds(d, HG, stride=PITCH), :]
                                for d in range(16 * half, 16 * half + 16)], axis=0)

    def prep_qkv(i2, carry):
        for e in range(PU):
            prep_qkv1(i2 * PU + e, 6 * e)
        return carry

    def prep_qkv1(i, t0):
        l, g, c = i // (4 * G), (i // 4) % G, i % 4
        for half in range(2):
            for part in range(3):
                scatter_heads(t0 + 3 * half + part, raw_qkv[
                    l, cols(c + 4 * half, 128), cols(part * G + g, GR)].astype(F32).T)
        for s in range(3):
            quad = [gather_dims(t0 + 3 * half + ROWS[s + 3 * mh][0], ROWS[s + 3 * mh][1])
                    for mh in range(2) for half in range(2)]
            for m, val in enumerate(lhs_operands(*quad)):
                wt[l, c, cols((g * 7 + m) * 3 + s, 64), :] = words(val)

    def prep_wo(i, carry):
        l, g = i // G, i % G
        for c in range(NC):
            scatter_heads(c, raw_wo[l, cols(g, GR), cols(c, 128)].astype(F32))
        for c in range(4):
            quad = [gather_dims(c + 4 * mh, half).astype(BF16).T.astype(F32)
                    for mh in range(2) for half in range(2)]
            for m, val in enumerate(lhs_operands(*quad)):
                wt[l, g, pl.ds(WO0 + m * (KH // 2) + c * 64, 64), :] = words(val)
        return carry

    def ln_pieces(p, z, j, LNS=LNS, LNC=LNC):
        def block(a, i, n):
            return x_get(p, j, a * D + i * n, n).reshape(n // 8, 8, 128)

        def total(v):
            return jnp.sum(jnp.sum(v.reshape(-1, 4, 8, 128), axis=0), axis=0)

        def stat(i):
            return x_get(p, j, ST0 + 8 * i, 8)

        def put_stat(i, val):
            x_put(p + z, j, ST0 + 8 * i, jnp.broadcast_to(val, (8, 128)))

        def mean(a, i):
            m = total(block(a, i, D // LNS))
            if i > 0:
                m = m + stat(4 + a)
            if i < LNS - 1:
                put_stat(4 + a, m)
            else:
                put_stat(a, jnp.sum(m, axis=0, keepdims=True) * (1.0 / D))

        def var(a, i):
            c = block(a, i, D // LNS) - stat(a)[None]
            v = total(c * c)
            if i > 0:
                v = v + stat(6 + a)
            if i < LNS - 1:
                put_stat(6 + a, v)
            else:
                v = jnp.sum(v, axis=0, keepdims=True) * (1.0 / D)
                put_stat(2 + a, jax.lax.rsqrt(v + EPS))

        def norm(i):
            n = KH // LNC
            quad = [((block(a, kh * LNC + i, n) - stat(a)[None]) * stat(2 + a)[None]).reshape(n, 128)
                    for kh in range(2) for a in range(2)]
            for m, val in enumerate(rhs_operands(*quad)):
                x_put(p + z, j, XN0 + (m * KH + i * n) // 2, words(val))

        stats = [[functools.partial(f, a, i) for f in (mean, var) for i in range(LNS)]
                 for a in range(2)]
        return stats[0], stats[1] + [functools.partial(norm, i) for i in range(LNC)]

    fbs = (fb0, fb1)

    def o_rows(j, m, g2):
        n = 7 * j + m
        return OB + n // 2, (n % 2) * 128 + g2 * 64

    def att_pieces(g2, z, par):
        src, dst = fbs[par], fbs[1 - par]
        lane0 = jax.lax.broadcasted_iota(jnp.int32, (8, 128), 1) == 0

        def qk(r, w0):
            acc = {}
            for d in range(DH):
                rs = slice(8 * d, 8 * d + 8)
                q = src[Q0 + r, rs, :]
                for w in range(w0, w0 + WQ):
                    t = q * src[K0 + r - w + W - 1, rs, :]
                    acc[w] = t if d == 0 else acc[w] + t
            lg = [jnp.where(lane0, -1e9, acc[w] * SCALE) if w > r else acc[w] * SCALE
                  for w in range(w0, w0 + WQ)]
            lg = jnp.concatenate(lg, axis=0)
            dst[z + PB + r % 2, w0 * 8:(w0 + WQ) * 8, :] = lg
            prob[r, w0 * 8:(w0 + WQ) * 8, :] = lg

        def softmax(r):
            lg = [prob[r, w * 8:w * 8 + 8, :] for w in range(W)]
            m = functools.reduce(jnp.maximum, lg)
            e = [jnp.exp(t - m) for t in lg]
            inv = 1.0 / functools.reduce(jnp.add, e)
            pr = jnp.concatenate([t * inv for t in e], axis=0)
            prob[r, 64:128, :] = pr

        def pv(j, c):
            quad = []
            for kh in range(2):
                rs = slice(kh * 128 + 16 * c, kh * 128 + 16 * c + 16)
                v = [src[V0 + 2 * j + e, rs, :].reshape(2, 8, 128) for e in range(W + 1)]
                for a in range(2):
                    o = None
                    for w in range(W):
                        t = v[a - w + W - 1] * prob[2 * j + a, 64 + w * 8:72 + w * 8, :][None]
                        o = t if o is None else o + t
                    quad.append(o.reshape(16, 128))
            for m, val in enumerate(rhs_operands(*quad)):
                tile, row = o_rows(j, m, g2)
                dst[z + tile, pl.ds(pl.multiple_of(row + 8 * c, 8), 8), :] = words(val)

        def scores(j):
            out = []
            for r in (2 * j, 2 * j + 1):
                out += [functools.partial(qk, r, w0) for w0 in range(0, W, WQ)]
                out[-1] = functools.partial(run, [out[-1], functools.partial(softmax, r)])
            return out

        pieces = []
        for j in range(NP):
            pieces += scores(j) + [functools.partial(pv, j, c) for c in range(8)]
        return pieces

    def spread(pieces, weights):
        total = float(sum(weights))
        state = [0, 0.0, 0]

        def fill():
            state[1] += weights[state[0]]
            state[0] += 1
            while state[2] < min(len(pieces), int(state[1] * len(pieces) / total + 0.5)):
                pieces[state[2]]()
                state[2] += 1
        return fill

    def run(pieces):
        for f in pieces:
            f()

    def lhs(l, rows):
        return jnp.concatenate(
            [pltpu.bitcast(wt[l, c, rows, :], BF16) for c in range(4)], axis=1)

    def qkv_step(l, p, g, par, att):
        fb = fbs[par]
        q0, k0, v0 = Q0, K0, V0
        fill = spread(att, [1] * (NP * 7 * (HM // SR)))
        lane0 = jax.lax.broadcasted_iota(jnp.int32, (SR, 128), 1) == 0

        def final(row, r, val):
            part, r0 = ROWS[row // 128][0], ROWS[row // 128][1] * 128 + row % 128
            rr = slice(r0, r0 + SR)
            if part == 0:
                fb[q0 + r, rr, :] = val
            elif part == 1:
                fb[k0 + W - 1 + r, rr, :] = val
                if r > 0:
                    fb[k0 + r - 1, rr, :] = pltpu.roll(val, 1, 1)
            else:
                fb[v0 + W - 1 + r, rr, :] = val
                if r == 0:
                    vfirst[g, rr, :] = jnp.where(p == 0, val, vfirst[g, rr, :])
                else:
                    fb[v0 + r - 1, rr, :] = jnp.where(
                        lane0, vfirst[g, rr, :], pltpu.roll(val, 1, 1))

        for j in range(NP):
            for m in (0, 1, 2, 5, 3, 4, 6):
                res = jnp.dot(lhs(l, cols(g * 7 + m, HM // 2)),
                              pltpu.bitcast(x_get(p, j, XN0 + m * KH // 2, KH // 2), BF16),
                              preferred_element_type=F32)
                for s0 in range(0, HM, SR):
                    val = res[s0:s0 + SR]
                    t1, t2, t3, tx, ty = [
                        (TMP + 2 * t + s0 // GR, slice(s0 % GR, s0 % GR + SR), slice(None))
                        for t in range(5)]
                    if m == 0:
                        fb[t1] = val
                    elif m == 1:
                        fb[t2] = val
                    elif m == 2:
                        fb[tx] = fb[t1] - fb[t2] + val
                        fb[t3] = val
                    elif m == 5:
                        final(HM + s0, 2 * j + 1, fb[tx] + val)
                    elif m == 3:
                        final(HM + s0, 2 * j, fb[t2] + val)
                        fb[ty] = fb[t1] + val
                    elif m == 4:
                        final(s0, 2 * j + 1, fb[t3] + val)
                        fb[ty] = fb[ty] - val
                    else:
                        final(s0, 2 * j, fb[ty] + val)
                    fill()

    feeds = (((0, 0, 1), (1, 1, 1)), ((1, 0, 1), (1, 1, -1)), ((0, 1, 1), (1, 1, 1)),
             ((0, 0, 1), (1, 0, 1)), ((0, 0, -1), (0, 1, 1)), ((1, 1, 1),), ((0, 0, 1),))

    def o_operand(j, m):
        parts = []
        for g in range(G):
            tile, row = o_rows(j, m, g // 2)
            parts.append(pltpu.bitcast(fbs[1 - g % 2][tile, row:row + 64, :], BF16))
        return jnp.concatenate(parts, axis=0)

    def wo_step(l, p, z, more):
        n = KH // SW
        for j in range(NP):
            fill = spread(sum(ln_pieces(p, z, j - 1), []) if j > 0 else [], [1] * (7 * n))
            head = ln_pieces(p, z, j)[0] if j == NP - 1 else []
            fill_head = spread(head, [1] * (2 * n))
            for mi, m in enumerate((0, 1, 3, 4, 6, 2, 5)):
                res = jnp.dot(lhs(l, pl.ds(WO0 + m * (KH // 2), KH // 2)),
                              o_operand(j, m),
                              preferred_element_type=F32)
                for s0 in range(0, KH, SW):
                    for mh, a, sign in feeds[m]:
                        r0 = a * D + mh * KH + s0
                        old, val = x_get(p, j, r0, SW), res[s0:s0 + SW]
                        x_put(p, j, r0, old + val if sign > 0 else old - val)
                    fill()
                    if mi >= 5:
                        fill_head()
        pl.when(more)(functools.partial(run, ln_pieces(p, 0, NP - 1, RS, RC)[1]))

    def prep_a_group(g):
        for part in range(3):
            cp_a(g, part).wait()
        jax.lax.fori_loop(4 * g // PU, (4 * g + 4) // PU, prep_qkv, 0)

    vfirst[...] = jnp.zeros_like(vfirst)
    tmp[...] = jnp.zeros_like(tmp)
    fb1[0:TMP] = jnp.zeros((TMP, GR, 128), F32)
    prep_x(0, 0, first=True)
    jax.lax.fori_loop(1, NC, prep_x, 0)
    jax.lax.fori_loop(0, 2 * NP, first_norm, 0)
    prep_a_group(0)

    def body(i, carry):
        u, h = i // 2, i % 2
        p = u % 2
        l = (u // 2) % 2
        z = (i * i) // 512

        @pl.when(i == 1)
        def _():
            for g in (2, 3):
                for part in range(3):
                    cp_a(g, part).wait()

        @pl.when(i == 2)
        def _():
            for c in cp_rest:
                c.wait()
            jax.lax.fori_loop(0, 2 * G, prep_wo, 0)

        @pl.when(jnp.logical_or(i == 1, i == 2))
        def _():
            jax.lax.fori_loop(8 * i // PU, 16 * i // PU, prep_qkv, 0)

        @pl.when(i < 16)
        def _():
            qkv_step(l, p, 2 * h, 0, att_pieces(1 - h, z, 1))

        @pl.when(i == 16)
        def _():
            run(att_pieces(1, 0, 1))

        @pl.when(jnp.logical_and(h == 0, i > 0))
        def _():
            wo_step(((u - 1) // 2) % 2, 1 - p, z, u < 7)

        @pl.when(i == 0)
        def _():
            prep_a_group(1)

        @pl.when(i < 16)
        def _():
            qkv_step(l, p, 2 * h + 1, 1, att_pieces(h, z, 0))
        return carry
    jax.lax.fori_loop(0, 17, body, 0)

    def cp_o(c):
        return pltpu.make_async_copy(out_st.at[c], out_hbm.at[:, cols(c, 128)], sems.at[c])

    def emit(c, carry):
        ou = out_st.bitcast(U32)
        for r in range(NB):
            wd = pack(*(x_get(p, r // 2, r % 2 * D + c * 128, 128) for p in range(2)))
            ou[c, pl.ds(r, 128, stride=NB), :] = pltpu.bitcast(wd.T, U32)
        cp_o(c).start()
        return carry
    jax.lax.fori_loop(0, NC, emit, 0)
    for c in range(NC):
        cp_o(c).wait()


def scratch_shapes():
    return [
        pltpu.VMEM((NC, S, 128), BF16),
        pltpu.VMEM((2, D, 3 * D), BF16),
        pltpu.VMEM((2, D, D), BF16),
        pltpu.VMEM((2, 4, WO0 + 7 * KH // 2, 128), F32),
        pltpu.VMEM((6 * PU, HG * PITCH, 128), F32),
        pltpu.VMEM((2, NP, ST0 + 64, 128), F32),
        pltpu.VMEM((NT, GR, 128), F32),
        pltpu.VMEM((NT, GR, 128), F32),
        pltpu.VMEM((NB, 128, 128), F32),
        pltpu.VMEM((2, NB, 4, 8, 128), F32),
        pltpu.VMEM((G, GR, 128), F32),
        pltpu.VMEM((NC, S, 128), BF16),
        pltpu.SemaphoreType.DMA((24,)),
    ]


@jax.jit
def pallas_interleave_layers__sliding_local_dilated__sliding_local_dilated__prompt_kernel(
    A_x: jax.Array,
    A_wqkv: jax.Array,
    A_wo: jax.Array,
    B_x: jax.Array,
    B_wqkv: jax.Array,
    B_wo: jax.Array,
):
    del B_x
    any_spec = pl.BlockSpec(memory_space=pl.ANY)
    out = pl.pallas_call(
        kernel,
        out_shape=jax.ShapeDtypeStruct((S, D), BF16),
        in_specs=[any_spec] * 5,
        out_specs=any_spec,
        scratch_shapes=scratch_shapes(),
        compiler_params=pltpu.CompilerParams(vmem_limit_bytes=112 * 1024 * 1024),
    )(A_x.reshape(S, D), A_wqkv, A_wo, B_wqkv, B_wo)
    return out.reshape(1, S, D)
```

```python
import functools

import jax
import jax.numpy as jnp
from jax.experimental import pallas as pl
from jax.experimental.pallas import tpu as pltpu

S, D, H, DH, W = 2048, 1024, 32, 32, 8
T = S // 2
NB = T // 128
NP = NB // 2
NC = D // 128
G = 4
GR = D // G
HG = GR // DH
NE = NB + W - 1
KH = D // 2
HM = 3 * GR // 2
F32, BF16, U32 = jnp.float32, jnp.bfloat16, jnp.uint32
EPS = 1e-5
SCALE = DH ** -0.5
ROWS = ((1, 0), (0, 0), (0, 1), (1, 1), (2, 0), (2, 1))
PITCH = DH + 1
Q0, K0, V0 = 0, NB, NB + NE
TMP = NB + 2 * NE
PB = TMP + 10
OB = PB + 2
NT = OB + 7 * NP // 2
XN0 = 2 * D
ST0 = XN0 + 7 * KH // 2
WO0 = G * 7 * HM // 2


def lhs_operands(a11, a12, a21, a22):
    return (a11 + a22, a21 + a22, a11, a22, a11 + a12, a21 - a11, a12 - a22)


def rhs_operands(b11, b12, b21, b22):
    return (b11 + b22, b11, b12 - b22, b21 - b11, b22, b11 + b12, b21 + b22)


WQ = 4
SR, SW = 32, 32
LNS, LNC = 4, 32
RS, RC = 4, 16
PU = 4


def kernel(x_hbm, aqkv_hbm, awo_hbm, bqkv_hbm, bwo_hbm, out_hbm,
           x_raw, raw_qkv, raw_wo, wt, tmp, xs, xn_last, fb0, fb1, prob, moments, vfirst, out_st, sems):
    def cols(i, n):
        return pl.ds(i * n if isinstance(i, int) else pl.multiple_of(i * n, n), n)

    def cp_x(c):
        return pltpu.make_async_copy(x_hbm.at[:, cols(c, 128)], x_raw.at[c, pl.ds(0, S)],
                                     sems.at[c])

    def cp_a(g, part):
        cs = cols(part * G + g, GR)
        return pltpu.make_async_copy(aqkv_hbm.at[:, cs], raw_qkv.at[0, :, cs],
                                     sems.at[NC + 3 * g + part])

    cp_rest = [pltpu.make_async_copy(awo_hbm, raw_wo.at[0], sems.at[NC + 12]),
               pltpu.make_async_copy(bqkv_hbm, raw_qkv.at[1], sems.at[NC + 13]),
               pltpu.make_async_copy(bwo_hbm, raw_wo.at[1], sems.at[NC + 14])]
    for c in range(NC):
        cp_x(c).start()
    for g in range(G):
        for part in range(3):
            cp_a(g, part).start()
    for c in cp_rest:
        c.start()

    def x_rows(r0, n):
        return pl.ds(r0 if isinstance(r0, int) else pl.multiple_of(r0, 8), n)

    def x_get(p, j, r0, n):
        return xs[p, j, x_rows(r0, n), :]

    def x_put(p, j, r0, val):
        xs[p, j, x_rows(r0, val.shape[0]), :] = val

    def lane_mean(v, n):
        return jnp.broadcast_to(jnp.sum(v, axis=0, keepdims=True) * (1.0 / n), (8, 128))

    def prep_x(c, carry, first=False):
        xu = x_raw.bitcast(U32)
        cp_x(c).wait()
        for r in range(NB):
            j, a = r // 2, r % 2
            wd = xu[c, pl.ds(r, 128, stride=NB), :]
            for p, val in enumerate(halves(pltpu.bitcast(wd, F32).T)):
                x_put(p, j, a * D + c * 128, val)
                val = val.reshape(16, 8, 128)
                if first:
                    shift = lane_mean(jnp.sum(val, axis=0), 128)
                    moments[p, r, 2] = shift
                else:
                    shift = moments[p, r, 2]
                dv = val - shift[None]
                for i, t in enumerate((jnp.sum(dv, axis=0), jnp.sum(dv * dv, axis=0))):
                    moments[p, r, i] = t if first else moments[p, r, i] + t
        return carry

    def first_norm(i, carry, last=False):
        p, j = (i, NP - 1) if last else (i // (NP - 1), i % (NP - 1))
        for a in range(2):
            m = lane_mean(moments[p, 2 * j + a, 0], D)
            v = jnp.maximum(lane_mean(moments[p, 2 * j + a, 1], D) - m * m, 0.0)
            x_put(p, j, ST0 + 8 * a, moments[p, 2 * j + a, 2] + m)
            x_put(p, j, ST0 + 8 * (2 + a), jax.lax.rsqrt(v + EPS))
        run(ln_pieces(p, 0, j, 1, RC, last)[1][-RC:])
        return carry

    def words(val):
        return pltpu.bitcast(val.astype(BF16), F32)

    def halves(wd):
        wd = pltpu.bitcast(wd, U32)
        return (pltpu.bitcast(wd << 16, F32),
                pltpu.bitcast(wd & jnp.uint32(0xFFFF0000), F32))

    def pack(lo, hi):
        lo, hi = (pltpu.bitcast(t.astype(BF16).astype(F32), U32) for t in (lo, hi))
        return pltpu.bitcast((lo >> 16) | hi, F32)

    def scatter_heads(t, val):
        for h in range(HG):
            tmp[t, h * PITCH:h * PITCH + DH, :] = val[h * DH:(h + 1) * DH]

    def gather_dims(t, half):
        return jnp.concatenate([tmp[t, pl.ds(d, HG, stride=PITCH), :]
                                for d in range(16 * half, 16 * half + 16)], axis=0)

    def prep_qkv(i2, carry):
        for e in range(PU):
            prep_qkv1(i2 * PU + e, 6 * e)
        return carry

    def prep_qkv1(i, t0):
        l, g, c = i // (4 * G), (i // 4) % G, i % 4
        for half in range(2):
            for part in range(3):
                scatter_heads(t0 + 3 * half + part, raw_qkv[
                    l, cols(c + 4 * half, 128), cols(part * G + g, GR)].astype(F32).T)
        for s in range(3):
            quad = [gather_dims(t0 + 3 * half + ROWS[s + 3 * mh][0], ROWS[s + 3 * mh][1])
                    for mh in range(2) for half in range(2)]
            for m, val in enumerate(lhs_operands(*quad)):
                wt[l, c, cols((g * 7 + m) * 3 + s, 64), :] = words(val)

    def prep_wo(i, carry):
        l, g = i // G, i % G
        for c in range(NC):
            scatter_heads(c, raw_wo[l, cols(g, GR), cols(c, 128)].astype(F32))
        for c in range(4):
            quad = [gather_dims(c + 4 * mh, half).astype(BF16).T.astype(F32)
                    for mh in range(2) for half in range(2)]
            for m, val in enumerate(lhs_operands(*quad)):
                wt[l, g, pl.ds(WO0 + m * (KH // 2) + c * 64, 64), :] = words(val)
        return carry

    def ln_pieces(p, z, j, LNS=LNS, LNC=LNC, last=False):
        def block(a, i, n):
            return x_get(p, j, a * D + i * n, n).reshape(n // 8, 8, 128)

        def total(v):
            return jnp.sum(jnp.sum(v.reshape(-1, 4, 8, 128), axis=0), axis=0)

        def stat(i):
            return x_get(p, j, ST0 + 8 * i, 8)

        def put_stat(i, val):
            x_put(p + z, j, ST0 + 8 * i, jnp.broadcast_to(val, (8, 128)))

        def mean(a, i):
            m = total(block(a, i, D // LNS))
            if i > 0:
                m = m + stat(4 + a)
            if i < LNS - 1:
                put_stat(4 + a, m)
            else:
                put_stat(a, jnp.sum(m, axis=0, keepdims=True) * (1.0 / D))

        def var(a, i):
            c = block(a, i, D // LNS) - stat(a)[None]
            v = total(c * c)
            if i > 0:
                v = v + stat(6 + a)
            if i < LNS - 1:
                put_stat(6 + a, v)
            else:
                v = jnp.sum(v, axis=0, keepdims=True) * (1.0 / D)
                put_stat(2 + a, jax.lax.rsqrt(v + EPS))

        def norm(i):
            n = KH // LNC
            quad = [((block(a, kh * LNC + i, n) - stat(a)[None]) * stat(2 + a)[None]).reshape(n, 128)
                    for kh in range(2) for a in range(2)]
            for m, val in enumerate(rhs_operands(*quad)):
                if last:
                    xn_last[p, m * KH + i * n:m * KH + (i + 1) * n, :] = val.astype(BF16)
                else:
                    x_put(p + z, j, XN0 + (m * KH + i * n) // 2, words(val))

        stats = [[functools.partial(f, a, i) for f in (mean, var) for i in range(LNS)]
                 for a in range(2)]
        return stats[0], stats[1] + [functools.partial(norm, i) for i in range(LNC)]

    fbs = (fb0, fb1)

    def o_rows(j, m, g2):
        n = 7 * j + m
        return OB + n // 2, (n % 2) * 128 + g2 * 64

    def att_pieces(g2, z, par):
        src, dst = fbs[par], fbs[1 - par]
        lane0 = jax.lax.broadcasted_iota(jnp.int32, (8, 128), 1) == 0

        def qk(r, w0):
            acc = {}
            for d in range(DH):
                rs = slice(8 * d, 8 * d + 8)
                q = src[Q0 + r, rs, :]
                for w in range(w0, w0 + WQ):
                    t = q * src[K0 + r - w + W - 1, rs, :]
                    acc[w] = t if d == 0 else acc[w] + t
            lg = [jnp.where(lane0, -1e9, acc[w] * SCALE) if w > r else acc[w] * SCALE
                  for w in range(w0, w0 + WQ)]
            lg = jnp.concatenate(lg, axis=0)
            dst[z + PB + r % 2, w0 * 8:(w0 + WQ) * 8, :] = lg
            prob[r, w0 * 8:(w0 + WQ) * 8, :] = lg

        def softmax(r):
            lg = [prob[r, w * 8:w * 8 + 8, :] for w in range(W)]
            m = functools.reduce(jnp.maximum, lg)
            e = [jnp.exp(t - m) for t in lg]
            inv = 1.0 / functools.reduce(jnp.add, e)
            pr = jnp.concatenate([t * inv for t in e], axis=0)
            prob[r, 64:128, :] = pr

        def pv(j, c):
            quad = []
            for kh in range(2):
                rs = slice(kh * 128 + 16 * c, kh * 128 + 16 * c + 16)
                v = [src[V0 + 2 * j + e, rs, :].reshape(2, 8, 128) for e in range(W + 1)]
                for a in range(2):
                    o = None
                    for w in range(W):
                        t = v[a - w + W - 1] * prob[2 * j + a, 64 + w * 8:72 + w * 8, :][None]
                        o = t if o is None else o + t
                    quad.append(o.reshape(16, 128))
            for m, val in enumerate(rhs_operands(*quad)):
                tile, row = o_rows(j, m, g2)
                dst[z + tile, pl.ds(pl.multiple_of(row + 8 * c, 8), 8), :] = words(val)

        def scores(j):
            out = []
            for r in (2 * j, 2 * j + 1):
                out += [functools.partial(qk, r, w0) for w0 in range(0, W, WQ)]
                out[-1] = functools.partial(run, [out[-1], functools.partial(softmax, r)])
            return out

        pieces = []
        for j in range(NP):
            pieces += scores(j) + [functools.partial(pv, j, c) for c in range(8)]
        return pieces

    def spread(pieces, weights):
        total = float(sum(weights))
        state = [0, 0.0, 0]

        def fill():
            state[1] += weights[state[0]]
            state[0] += 1
            while state[2] < min(len(pieces), int(state[1] * len(pieces) / total + 0.5)):
                pieces[state[2]]()
                state[2] += 1
        return fill

    def run(pieces):
        for f in pieces:
            f()

    def lhs(l, rows):
        return jnp.concatenate(
            [pltpu.bitcast(wt[l, c, rows, :], BF16) for c in range(4)], axis=1)

    def xn_operand(p, j, m):
        if j == NP - 1:
            return xn_last[p, m * KH:(m + 1) * KH, :]
        return pltpu.bitcast(x_get(p, j, XN0 + m * KH // 2, KH // 2), BF16)

    def qkv_step(l, p, g, par, att):
        fb = fbs[par]
        q0, k0, v0 = Q0, K0, V0
        fill = spread(att, [1] * (NP * 7 * (HM // SR)))
        lane0 = jax.lax.broadcasted_iota(jnp.int32, (SR, 128), 1) == 0

        def final(row, r, val):
            part, r0 = ROWS[row // 128][0], ROWS[row // 128][1] * 128 + row % 128
            rr = slice(r0, r0 + SR)
            if part == 0:
                fb[q0 + r, rr, :] = val
            elif part == 1:
                fb[k0 + W - 1 + r, rr, :] = val
                if r > 0:
                    fb[k0 + r - 1, rr, :] = pltpu.roll(val, 1, 1)
            else:
                fb[v0 + W - 1 + r, rr, :] = val
                if r == 0:
                    vfirst[g, rr, :] = jnp.where(p == 0, val, vfirst[g, rr, :])
                else:
                    fb[v0 + r - 1, rr, :] = jnp.where(
                        lane0, vfirst[g, rr, :], pltpu.roll(val, 1, 1))

        for j in range(NP):
            for m in ((0, 1, 2, 3, 5, 4, 6) if j == 0 else (0, 1, 2, 5, 3, 4, 6)):
                res = jnp.dot(lhs(l, cols(g * 7 + m, HM // 2)),
                              xn_operand(p, j, m),
                              preferred_element_type=F32)
                for s0 in range(0, HM, SR):
                    val = res[s0:s0 + SR]
                    t1, t2, t3, tx, ty = [
                        (TMP + 2 * t + s0 // GR, slice(s0 % GR, s0 % GR + SR), slice(None))
                        for t in range(5)]
                    if m == 0:
                        fb[t1] = val
                    elif m == 1:
                        fb[t2] = val
                    elif m == 2:
                        fb[tx] = fb[t1] - fb[t2] + val
                        fb[t3] = val
                    elif m == 5:
                        final(HM + s0, 2 * j + 1, fb[tx] + val)
                    elif m == 3:
                        final(HM + s0, 2 * j, fb[t2] + val)
                        fb[ty] = fb[t1] + val
                    elif m == 4:
                        final(s0, 2 * j + 1, fb[t3] + val)
                        fb[ty] = fb[ty] - val
                    else:
                        final(s0, 2 * j, fb[ty] + val)
                    fill()

    feeds = (((0, 0, 1), (1, 1, 1)), ((1, 0, 1), (1, 1, -1)), ((0, 1, 1), (1, 1, 1)),
             ((0, 0, 1), (1, 0, 1)), ((0, 0, -1), (0, 1, 1)), ((1, 1, 1),), ((0, 0, 1),))

    def o_operand(j, m):
        parts = []
        for g in range(G):
            tile, row = o_rows(j, m, g // 2)
            parts.append(pltpu.bitcast(fbs[1 - g % 2][tile, row:row + 64, :], BF16))
        return jnp.concatenate(parts, axis=0)

    def wo_step(l, p, z, more):
        n = KH // SW
        for j in range(NP):
            fill = spread(sum(ln_pieces(p, z, j - 1), []) if j > 0 else [], [1] * (7 * n))
            head = ln_pieces(p, z, j)[0] if j == NP - 1 else []
            fill_head = spread(head, [1] * (2 * n))
            for mi, m in enumerate((0, 1, 3, 4, 6, 2, 5)):
                res = jnp.dot(lhs(l, pl.ds(WO0 + m * (KH // 2), KH // 2)),
                              o_operand(j, m),
                              preferred_element_type=F32)
                for s0 in range(0, KH, SW):
                    for mh, a, sign in feeds[m]:
                        r0 = a * D + mh * KH + s0
                        old, val = x_get(p, j, r0, SW), res[s0:s0 + SW]
                        x_put(p, j, r0, old + val if sign > 0 else old - val)
                    fill()
                    if mi >= 5:
                        fill_head()
        pl.when(more)(functools.partial(run, ln_pieces(p, 0, NP - 1, RS, RC, True)[1]))

    def prep_a_group(g):
        for part in range(3):
            cp_a(g, part).wait()
        jax.lax.fori_loop(4 * g // PU, (4 * g + 4) // PU, prep_qkv, 0)

    vfirst[...] = jnp.zeros_like(vfirst)
    tmp[...] = jnp.zeros_like(tmp)
    fb1[0:TMP] = jnp.zeros((TMP, GR, 128), F32)
    prep_x(0, 0, first=True)
    jax.lax.fori_loop(1, NC, prep_x, 0)
    jax.lax.fori_loop(0, 2 * (NP - 1), first_norm, 0)
    jax.lax.fori_loop(0, 2, functools.partial(first_norm, last=True), 0)
    prep_a_group(0)

    def body(i, carry):
        u, h = i // 2, i % 2
        p = u % 2
        l = (u // 2) % 2
        z = (i * i) // 512

        @pl.when(i == 1)
        def _():
            for g in (2, 3):
                for part in range(3):
                    cp_a(g, part).wait()

        @pl.when(i == 2)
        def _():
            for c in cp_rest:
                c.wait()
            jax.lax.fori_loop(0, 2 * G, prep_wo, 0)

        @pl.when(jnp.logical_or(i == 1, i == 2))
        def _():
            jax.lax.fori_loop(8 * i // PU, 16 * i // PU, prep_qkv, 0)

        @pl.when(i < 16)
        def _():
            qkv_step(l, p, 2 * h, 0, att_pieces(1 - h, z, 1))

        @pl.when(i == 16)
        def _():
            run(att_pieces(1, 0, 1))

        @pl.when(jnp.logical_and(h == 0, i > 0))
        def _():
            wo_step(((u - 1) // 2) % 2, 1 - p, z, u < 7)

        @pl.when(i == 0)
        def _():
            prep_a_group(1)

        @pl.when(i < 16)
        def _():
            qkv_step(l, p, 2 * h + 1, 1, att_pieces(h, z, 0))
        return carry
    jax.lax.fori_loop(0, 17, body, 0)

    def cp_o(c):
        return pltpu.make_async_copy(out_st.at[c, pl.ds(0, S)], out_hbm.at[:, cols(c, 128)],
                                     sems.at[c])

    def emit(c, carry):
        ou = out_st.bitcast(U32)
        for r in range(NB):
            wd = pack(*(x_get(p, r // 2, r % 2 * D + c * 128, 128) for p in range(2)))
            ou[c, pl.ds(r, 128, stride=NB), :] = pltpu.bitcast(wd.T, U32)
        cp_o(c).start()
        return carry
    jax.lax.fori_loop(0, NC, emit, 0)
    for c in range(NC):
        cp_o(c).wait()


def scratch_shapes():
    return [
        pltpu.VMEM((NC, S + 16, 128), BF16),
        pltpu.VMEM((2, D, 3 * D), BF16),
        pltpu.VMEM((2, D, D), BF16),
        pltpu.VMEM((2, 4, WO0 + 7 * KH // 2, 128), F32),
        pltpu.VMEM((6 * PU, HG * PITCH + DH, 128), F32),
        pltpu.VMEM((2, NP, ST0 + 64, 128), F32),
        pltpu.VMEM((2, 7 * KH, 128), BF16),
        pltpu.VMEM((NT, GR, 128), F32),
        pltpu.VMEM((NT, GR, 128), F32),
        pltpu.VMEM((NB, 128, 128), F32),
        pltpu.VMEM((2, NB, 4, 8, 128), F32),
        pltpu.VMEM((G, GR, 128), F32),
        pltpu.VMEM((NC, S + 16, 128), BF16),
        pltpu.SemaphoreType.DMA((24,)),
    ]


@jax.jit
def pallas_interleave_layers__sliding_local_dilated__sliding_local_dilated__prompt_kernel(
    A_x: jax.Array,
    A_wqkv: jax.Array,
    A_wo: jax.Array,
    B_x: jax.Array,
    B_wqkv: jax.Array,
    B_wo: jax.Array,
):
    del B_x
    any_spec = pl.BlockSpec(memory_space=pl.ANY)
    out = pl.pallas_call(
        kernel,
        out_shape=jax.ShapeDtypeStruct((S, D), BF16),
        in_specs=[any_spec] * 5,
        out_specs=any_spec,
        scratch_shapes=scratch_shapes(),
        compiler_params=pltpu.CompilerParams(vmem_limit_bytes=112 * 1024 * 1024),
    )(A_x.reshape(S, D), A_wqkv, A_wo, B_wqkv, B_wo)
    return out.reshape(1, S, D)
```
